```python
import os as _os
_os.environ.setdefault("JAX_PLATFORMS", "cpu")
import jax
import jax.numpy as jnp

def _softmax(x, axis=-1):
    return jax.nn.softmax(x, axis=axis)
def _gelu(x):
    return jax.nn.gelu(x, approximate=True)
def _silu(x):
    return jax.nn.silu(x)
def _sigmoid(x):
    return jax.nn.sigmoid(x)
def _layernorm(x, axis=-1, eps=1e-5):
    m = jnp.mean(x, axis=axis, keepdims=True)
    v = jnp.var(x, axis=axis, keepdims=True)
    return (x - m) / jnp.sqrt(v + eps)
def _scatter_add(tgt, idx, src, axis=0):
    return tgt.at[idx].add(src)
def _segment_sum(src, seg, n):
    return jax.ops.segment_sum(src, seg, n)
class _Rng:
    def __init__(self, key):
        self._k = key
    def _next(self):
        self._k, sub = jax.random.split(self._k)
        return sub
    def normal(self, shape):
        return jax.random.normal(self._next(), shape, dtype=jnp.bfloat16)
    def randint(self, lo, hi, shape):
        return jax.random.randint(self._next(), shape, lo, hi, dtype=jnp.int32)
    def uniform(self, shape, lo=0.0, hi=1.0):
        return jax.random.uniform(self._next(), shape, jnp.bfloat16, lo, hi)
    def permutation(self, n):
        return jax.random.permutation(self._next(), n)


kernel_name = 'recurrent_scan__sliding_block__dense_activation_mish__prompt'

def setup_inputs():
    _rng = _Rng(jax.random.key(int.from_bytes(__import__("os").urandom(4), "little")))
    _w = (lambda a: (lambda t: t.astype(jnp.bfloat16) if jnp.issubdtype(t.dtype, jnp.floating) else t)(jnp.asarray(a)))
    def _A_setup():
        B, S, D = 1, 2048, 576
        return {
            "x": _w((lambda *s: _rng.normal(s) * 0.05)(B, S, D)),
            "wqkv": _w((lambda *s: _rng.normal(s) * 0.1)(D, 3 * D)),
            "wo": _w((lambda *s: _rng.normal(s) * 0.1)(D, D)),
        }
    _A_in = _A_setup()

    def _B_setup():
        B, S, D, F = 1, 2048, 576, 4608
        return {
            "x": _w((lambda *s: _rng.normal(s) * 0.05)(B, S, D)),
            "w1": _w((lambda *s: _rng.normal(s) * 0.05)(D, F) * (D ** -0.5)),
            "b1": _w((lambda *s: _rng.normal(s) * 0.05)(F)),
            "w2": _w((lambda *s: _rng.normal(s) * 0.05)(F, D) * (F ** -0.5)),
        }
    _B_in = _B_setup()

    return {
        "A_x": _A_in["x"],
        "A_wqkv": _A_in["wqkv"],
        "A_wo": _A_in["wo"],
        "B_x": _B_in["x"],
        "B_w1": _B_in["w1"],
        "B_b1": _B_in["b1"],
        "B_w2": _B_in["w2"],
    }

def reference(A_x, A_wqkv, A_wo, B_x, B_w1, B_b1, B_w2):
    def _A_ref(x, wqkv, wo):
        B, S, D = x.shape
        H = 32; Dh = D // H; W = 256
        qkv = (lambda x, *d: x.transpose(*d))((x @ wqkv).reshape(B, S, 3, H, Dh), 2, 0, 3, 1, 4)
        q, k, v = qkv[0], qkv[1], qkv[2]
        scores = jnp.einsum("bhqd,bhkd->bhqk", q, k) * (Dh ** -0.5)
        idx = jnp.arange(S)
        mask = (idx[:, None] - idx[None, :] >= 0) & (idx[:, None] - idx[None, :] < W)
        scores = jnp.where(mask[None, None], scores, -1e9)
        p = _softmax(scores, axis=-1)
        o = jnp.einsum("bhqk,bhkd->bhqd", p, v)
        return (lambda x, *d: x.transpose(*d))(o, 0, 2, 1, 3).reshape(B, S, D) @ wo

    def _B_ref(x, w1, b1, w2):
        h = jnp.einsum("bsd,df->bsf", x, w1) + b1
        sp = jnp.log1p(jnp.exp(-jnp.abs(h))) + jnp.where(h > 0, h, jnp.zeros_like(h))
        act = h * jnp.tanh(sp)
        return jnp.einsum("bsf,fd->bsd", act, w2)

    x = A_x
    xn = _layernorm(x, axis=-1)
    s = _A_ref(xn, A_wqkv, A_wo)
    g = _silu(_B_ref(xn, B_w1, B_b1, B_w2))
    return x + s * g
```

```python
import jax
import jax.numpy as jnp
from jax import lax
import jax.experimental.pallas as pl
import jax.experimental.pallas.tpu as pltpu

S, D, F, H, DH, WIN = 2048, 576, 4608, 32, 18, 256
LOG2E = 1.4426950408889634
F32, BF16, U32 = jnp.float32, jnp.bfloat16, jnp.uint32
NT = (((1,), (1,)), ((), ()))

def recip(d):
    r = pl.reciprocal(d, approx=True)
    return r * (2.0 - d * r)

def make(TB=512, CF=2304, G=7, LA=1):
    NB = S // TB
    QB = TB // 128
    NC = F // CF

    def kern(xt_hbm, wqkv_hbm, wo_hbm, w1_hbm, b1_ref, w2t_hbm, o_hbm,
             x_s, o_s, wqkv_s, wo_s, w1_s, w2t_s, wqk_s, k_s, vt_s, q_s, ot_s, acc_s, st_s, xn_s, trim_s, b1_s, sems, osem):
        cp_x0 = pltpu.make_async_copy(xt_hbm.at[:, 0:TB], x_s.at[:, 0:TB], sems.at[0])
        cp_x1 = pltpu.make_async_copy(xt_hbm.at[:, TB:], x_s.at[:, TB:], sems.at[1])
        cp_qkv = pltpu.make_async_copy(wqkv_hbm, wqkv_s, sems.at[2])
        cp_wo = pltpu.make_async_copy(wo_hbm, wo_s, sems.at[3])
        def cp_w1(c):
            return pltpu.make_async_copy(w1_hbm.at[:, pl.ds(c * CF, CF)], w1_s.at[c], sems.at[4 + c])
        def cp_w2(c):
            return pltpu.make_async_copy(w2t_hbm.at[:, pl.ds(c * CF, CF)], w2t_s.at[c], sems.at[4 + NC + c])
        def cp_o(i):
            c0 = pl.multiple_of(i * TB, TB)
            return pltpu.make_async_copy(o_s.at[:, pl.ds(c0, TB)], o_hbm.at[:, pl.ds(c0, TB)], osem.at[0])

        def layernorm(i, TB=TB):
            c0 = pl.multiple_of(i * TB, TB)
            x = x_s[:, pl.ds(c0, TB)].astype(F32)
            mu = jnp.mean(x, axis=0, keepdims=True)
            xc = x - mu
            var = jnp.mean(xc * xc, axis=0, keepdims=True)
            xnt = (xc * lax.rsqrt(var + 1e-5)).astype(BF16)
            return xnt, xnt.T

        def gate(i, TB=TB, TBF=TB):
            c0 = pl.multiple_of(i * TB, TB)
            mlp = acc_s[...]
            y = st_s[...] * (mlp * jax.nn.sigmoid(mlp))
            o_s[:, pl.ds(c0, TB)] = (x_s[:, pl.ds(c0, TB)].astype(F32) + y).astype(BF16)

        cp_qkv.start(); cp_x0.start()
        lane = lax.broadcasted_iota(jnp.int32, (WIN, 128), 1)
        kpad = jnp.where(lane == 126, 1.0, 0.0).astype(BF16)
        for t in range(5):
            k_s[t, 0:WIN, :] = kpad
        vt_s[0] = jnp.zeros((D, 128), BF16)
        vt_s[1] = jnp.zeros((D, 128), BF16)
        ll = lax.broadcasted_iota(jnp.int32, (128, 128), 1)
        ss = lax.broadcasted_iota(jnp.int32, (128, 128), 0)
        trim_s[...] = pltpu.bitcast(jnp.where(ss <= ll, 0xFFFF, 0).astype(jnp.uint16), U32)
        for c in range(NC):
            b1_s[c] = b1_ref[...].astype(F32).reshape(1, F)[:, c * CF:(c + 1) * CF]
        cp_x0.wait()
        cp_qkv.wait()
        cp_w1(0).start()
        cp_w2(0).start()
        for t in range(5):
            wqk_s[:, 128 * t:128 * (t + 1)] = wqkv_s[:, 126 * t:126 * t + 128]
            wqk_s[:, 640 + 128 * t:640 + 128 * (t + 1)] = wqkv_s[:, D + 126 * t:D + 126 * t + 128]

        def body(step, carry):
            xnt, xn = layernorm(step)
            xn_s[...] = xn
            qk = jnp.dot(xn, wqk_s[...], preferred_element_type=F32)
            vt = jnp.dot(wqkv_s[:, 2 * D:3 * D].T, xnt, preferred_element_type=F32)
            row0 = pl.multiple_of(step * TB, TB)
            lane_tb = lax.broadcasted_iota(jnp.int32, (TB, 128), 1)
            for t in range(5):
                kt = qk[:, 640 + 128 * t:640 + 128 * (t + 1)]
                k_s[t, pl.ds(row0 + WIN, TB), :] = jnp.where(lane_tb >= 126, 0.0, kt).astype(BF16)
                q_s[t] = (qk[:, 128 * t:128 * (t + 1)] * (LOG2E * DH ** -0.5)).astype(BF16)
            for b in range(QB):
                vt_s[step * QB + 2 + b] = vt[:, 128 * b:128 * (b + 1)].astype(BF16)
            def attention(bs):
                lane = lax.broadcasted_iota(jnp.int32, (128, 128), 1)
                subl = lax.broadcasted_iota(jnp.int32, (128, 128), 0)
                tri = subl <= lane
                r8 = lax.broadcasted_iota(jnp.int32, (8, 128), 0)
                lane64 = lax.broadcasted_iota(jnp.int32, (64, 128), 1)
                qfill = jnp.where(lane64 == 126, U32(0xCE6ECE6E), U32(0))
                pieces = {}
                def stage_a(b, hs):
                    t = hs[0] // 7
                    qt = pltpu.bitcast(q_s[t, pl.ds(pl.multiple_of(128 * b, 128), 128), :], U32)
                    qm = jnp.concatenate([pltpu.bitcast(jnp.where((lane64 >= DH * (h % 7)) & (lane64 < DH * (h % 7 + 1)), qt, qfill), BF16) for h in hs], axis=0)
                    kk = k_s[t, pl.ds(pl.multiple_of(row0 + 128 * b, 128), 384), :]
                    km = jnp.concatenate([kk[256:320], kk[64:128], kk[128:256]], axis=0)
                    main = lax.dot_general(km, qm, NT, preferred_element_type=F32)
                    old = pltpu.bitcast(kk[0:64], U32)
                    newr = pltpu.roll(pltpu.bitcast(kk[320:384], U32), 64, 1)
                    qr = pltpu.roll(qt[32:64], 64, 1)
                    l32 = lane64[0:32]
                    comb = []
                    for sel, js in (((l32 < 54) | (l32 == 126), (0, 1, 2)), ((l32 >= 54) & (l32 < 72), (3,)), (l32 >= 72, (4, 5, 6))):
                        js = [j for j in js if j < len(hs)]
                        if not js:
                            continue
                        q2 = []
                        for j in js:
                            q2.append(jnp.where((l32 >= DH * j) & (l32 < DH * (j + 1)), qt[0:32], qfill[0:32] if j != 3 else U32(0)))
                            lr = (l32 + 64) & 127
                            q2.append(jnp.where((lr >= DH * j) & (lr < DH * (j + 1)), qr, U32(0)))
                        r = lax.dot_general(pltpu.bitcast(jnp.where(sel, old, newr), BF16), pltpu.bitcast(jnp.concatenate(q2, axis=0), BF16), NT, preferred_element_type=F32)
                        comb += [r[:, 128 * i:128 * (i + 1)] for i in range(len(js))]
                    return main, comb, b
                def stage_b(st_all, n):
                    out = []
                    for i in range(n):
                        st = st_all[0][:, 128 * i:128 * (i + 1)]
                        cb = st_all[1][i]
                        s_mid = st[128:256]
                        lo_old = cb if i != 3 else jnp.where(step * QB + st_all[2] >= 2, cb, -1e9)
                        s_cmb = jnp.concatenate([jnp.where(tri[0:64], st[0:64], lo_old), jnp.where(tri[64:128], cb, st[64:128])], axis=0)
                        m = jnp.max(jnp.maximum(s_mid, s_cmb), axis=0, keepdims=True)
                        p_mid = jnp.exp2(s_mid - m).astype(BF16)
                        p_cmb = pltpu.bitcast(jnp.exp2(s_cmb - m).astype(BF16), U32)
                        p_new = p_cmb & trim_s[...]
                        out.append((pltpu.bitcast(p_cmb ^ p_new, BF16), p_mid, pltpu.bitcast(p_new, BF16)))
                    return out
                def stage_c(b, hs, ps):
                    for h, pp in zip(hs, ps):
                        w0 = (DH * h) // 16 * 16
                        off = DH * h - w0
                        spare = 24 if off < 8 else 0
                        acc = None
                        for i, p in enumerate(pp):
                            vw = pltpu.bitcast(vt_s[step * QB + b + i, w0:w0 + 32, :], U32)
                            if spare == 0:
                                vw = jnp.concatenate([jnp.where(r8 < 4, U32(0x3F803F80), vw[0:8]), vw[8:16]], axis=0)
                            else:
                                vw = jnp.concatenate([vw[0:8], jnp.where(r8 >= 4, U32(0x3F803F80), vw[8:16])], axis=0)
                            r = jnp.dot(pltpu.bitcast(vw, BF16), p, preferred_element_type=F32)
                            acc = r if acc is None else acc + r
                        rl = recip(acc[spare:spare + 8])
                        v0 = (DH * h) // 8
                        for vi in range(v0, v0 + 3):
                            lo = vi * 8 - w0
                            val = acc[lo:lo + 8] * rl
                            if (b, vi) in pieces:
                                val = jnp.where(r8 < DH * h - 8 * vi, pieces.pop((b, vi)), val)
                            if vi * 8 + 8 <= DH * (h + 1):
                                ot_s[vi * 8:vi * 8 + 8, pl.ds(pl.multiple_of(128 * b, 128), 128)] = val
                            else:
                                pieces[(b, vi)] = val
                groups = []
                for b in bs:
                    for t in range(5):
                        hs = list(range(7 * t, min(7 * t + 7, H)))
                        for i in range(0, len(hs), G):
                            groups.append((b, hs[i:i + G]))
                sa = {}
                n = len(groups)
                for u in range(n + LA):
                    if u < n:
                        sa[u] = stage_a(*groups[u])
                    if u >= LA:
                        stage_c(*groups[u - LA], stage_b(sa.pop(u - LA), len(groups[u - LA][1])))
                assert not pieces

            attention(list(range(QB)))
            acc_s[...] = jnp.zeros((D, TB), F32)

            def chunk(c, carry):
                @pl.when(step == 0)
                def _():
                    cp_w1(c).wait()
                    cp_w2(c).wait()
                    @pl.when(c + 1 < NC)
                    def _():
                        cp_w1(c + 1).start()
                        cp_w2(c + 1).start()
                    @pl.when(c == 0)
                    def _():
                        cp_wo.start(); cp_x1.start()
                    @pl.when(c == NC - 1)
                    def _():
                        cp_wo.wait(); cp_x1.wait()
                hh = jnp.dot(xn_s[...], w1_s[c], preferred_element_type=F32)
                hh = hh + b1_s[c]
                e = jnp.exp(jnp.minimum(hh, 20.0))
                n = e * (e + 2.0)
                act = (hh * n * recip(n + 2.0)).astype(BF16)
                acc_s[...] += lax.dot_general(w2t_s[c], act, NT, preferred_element_type=F32)
                return carry
            lax.fori_loop(0, NC, chunk, 0)
            st_s[...] = jnp.dot(wo_s[...].T, ot_s[...].astype(BF16), preferred_element_type=F32)
            gate(step)
            cp_o(step).start()
            return carry
        lax.fori_loop(0, NB, body, 0)
        pltpu.make_async_copy(o_s.at[:, 0:S], o_hbm, osem.at[0]).wait()

    def fn(A_x, A_wqkv, A_wo, B_x, B_w1, B_b1, B_w2):
        xt = A_x.reshape(S, D).T
        b1 = B_b1
        hbm = pl.BlockSpec(memory_space=pltpu.HBM)
        out = pl.pallas_call(
            kern,
            in_specs=[hbm, hbm, hbm, hbm, pl.BlockSpec(memory_space=pltpu.VMEM), hbm],
            out_specs=hbm,
            out_shape=jax.ShapeDtypeStruct((D, S), BF16),
            scratch_shapes=[
                pltpu.VMEM((D, S), BF16), pltpu.VMEM((D, S), BF16),
                pltpu.VMEM((D, 3 * D), BF16), pltpu.VMEM((D, D), BF16),
                pltpu.VMEM((NC, D, CF), BF16), pltpu.VMEM((NC, D, CF), BF16),
                pltpu.VMEM((D, 1280), BF16),
                pltpu.VMEM((5, S + WIN, 128), BF16),
                pltpu.VMEM((S // 128 + 2, D, 128), BF16), pltpu.VMEM((5, TB, 128), BF16),
                pltpu.VMEM((D, TB), F32), pltpu.VMEM((D, TB), F32), pltpu.VMEM((D, TB), F32),
                pltpu.VMEM((TB, D), BF16), pltpu.VMEM((64, 128), U32), pltpu.VMEM((NC, 1, CF), F32),
                pltpu.SemaphoreType.DMA((4 + 2 * NC,)), pltpu.SemaphoreType.DMA((1,))],
            compiler_params=pltpu.CompilerParams(vmem_limit_bytes=100 * 2**20),
            name="kmain",
        )(xt, A_wqkv, A_wo, B_w1, b1, B_w2.T)
        return out.T.reshape(1, S, D)
    return fn


@jax.jit
def pallas_recurrent_scan__sliding_block__dense_activation_mish__prompt_kernel(
    A_x, A_wqkv, A_wo, B_x, B_w1, B_b1, B_w2
):
    return make()(A_x, A_wqkv, A_wo, B_x, B_w1, B_b1, B_w2)
```
